```python
import os as _os
_os.environ.setdefault("JAX_PLATFORMS", "cpu")
import jax
import jax.numpy as jnp

def _softmax(x, axis=-1):
    return jax.nn.softmax(x, axis=axis)
def _gelu(x):
    return jax.nn.gelu(x, approximate=True)
def _silu(x):
    return jax.nn.silu(x)
def _sigmoid(x):
    return jax.nn.sigmoid(x)
def _layernorm(x, axis=-1, eps=1e-5):
    m = jnp.mean(x, axis=axis, keepdims=True)
    v = jnp.var(x, axis=axis, keepdims=True)
    return (x - m) / jnp.sqrt(v + eps)
def _scatter_add(tgt, idx, src, axis=0):
    return tgt.at[idx].add(src)
def _segment_sum(src, seg, n):
    return jax.ops.segment_sum(src, seg, n)
class _Rng:
    def __init__(self, key):
        self._k = key
    def _next(self):
        self._k, sub = jax.random.split(self._k)
        return sub
    def normal(self, shape):
        return jax.random.normal(self._next(), shape, dtype=jnp.bfloat16)
    def randint(self, lo, hi, shape):
        return jax.random.randint(self._next(), shape, lo, hi, dtype=jnp.int32)
    def uniform(self, shape, lo=0.0, hi=1.0):
        return jax.random.uniform(self._next(), shape, jnp.bfloat16, lo, hi)
    def permutation(self, n):
        return jax.random.permutation(self._next(), n)


kernel_name = 'gated_mix__mha_block__softmax_full_mha__prompt'

def setup_inputs():
    _rng = _Rng(jax.random.key(int.from_bytes(__import__("os").urandom(4), "little")))
    _w = (lambda a: (lambda t: t.astype(jnp.bfloat16) if jnp.issubdtype(t.dtype, jnp.floating) else t)(jnp.asarray(a)))
    def _A_setup():
        B, S, D, H = 1, 2048, 448, 16
        return {
            "x": _w((lambda *s: _rng.normal(s) * 0.05)(B, S, D)),
            "wqkv": _w((lambda *s: _rng.normal(s) * 0.4)(D, 3 * D)),
            "wo": _w((lambda *s: _rng.normal(s) * 0.05)(D, D)),
        }
    _A_in = _A_setup()

    def _B_setup():
        B, S, D = 1, 2048, 448
        return {
            "x": _w((lambda *s: _rng.normal(s) * 0.05)(B, S, D)),
            "wqkv": _w((lambda *s: _rng.normal(s) * 0.4)(D, 3 * D)),
            "wo": _w((lambda *s: _rng.normal(s) * 0.05)(D, D)),
        }
    _B_in = _B_setup()

    return {
        "A_x": _A_in["x"],
        "A_wqkv": _A_in["wqkv"],
        "A_wo": _A_in["wo"],
        "B_x": _B_in["x"],
        "B_wqkv": _B_in["wqkv"],
        "B_wo": _B_in["wo"],
        "gate_w": _w((lambda *s: _rng.normal(s) * 0.05)(448) * 16.0),
    }

def reference(A_x, A_wqkv, A_wo, B_x, B_wqkv, B_wo, gate_w):
    def _A_ref(x, wqkv, wo):
        B, S, D = x.shape
        H = 16
        Dh = D // H
        qkv = (lambda x, *d: x.transpose(*d))((x @ wqkv).reshape(B, S, 3, H, Dh), 2, 0, 3, 1, 4)
        q, k, v = qkv[0], qkv[1], qkv[2]
        scores = jnp.einsum("bhqd,bhkd->bhqk", q, k) * (Dh ** -0.5)
        p = _softmax(scores, axis=-1)
        o = jnp.einsum("bhqk,bhkd->bhqd", p, v)
        return (lambda x, *d: x.transpose(*d))(o, 0, 2, 1, 3).reshape(B, S, D) @ wo

    def _B_ref(x, wqkv, wo):
        B, S, D = x.shape
        H = 16; Dh = D // H
        qkv = (lambda x, *d: x.transpose(*d))((x @ wqkv).reshape(B, S, 3, H, Dh), 2, 0, 3, 1, 4)
        q, k, v = qkv[0], qkv[1], qkv[2]
        scale = Dh ** -0.5
        scores = jnp.einsum("bhqd,bhkd->bhqk", q, k) * scale
        p = _softmax(scores, axis=-1)
        o = jnp.einsum("bhqk,bhkd->bhqd", p, v)
        return (lambda x, *d: x.transpose(*d))(o, 0, 2, 1, 3).reshape(B, S, D) @ wo

    x = A_x
    g = _sigmoid((x * gate_w).sum(-1, keepdims=True))
    a = _A_ref(x, A_wqkv, A_wo)
    b = _B_ref(x, B_wqkv, B_wo)
    return g * a + (1 - g) * b
```

```python
import jax
import jax.numpy as jnp
from jax import lax
import jax.experimental.pallas as pl
import jax.experimental.pallas.tpu as pltpu

S, D, H, DH = 2048, 448, 16, 28
HP = 32
DP = H * HP
NSLAB = DP // 128
F3 = 3 * D
GR = 16
FR = F3 + GR
QSCALE = float(DH ** -0.5 * 1.4426950408889634)
F32, BF16 = jnp.float32, jnp.bfloat16


def _pad_heads(ref, base, cols):
    return jnp.concatenate([ref[pl.ds(base + DH * h, HP), cols] for h in range(H)], axis=0)


def make_kernel(TQ=1024, SQ=512, CK=128, CH=512, flags=None, defer=True):
    NQ = S // TQ
    NC = S // CK
    NT_ = 2 * H
    NCH = S // CH
    NU = TQ // SQ

    def kernel(x_hbm, awqkv_hbm, awo_hbm, bwqkv_hbm, bwo_hbm, gw_ref, out_ref,
               x_scr, w_scr, wo_scr, wt_scr, y_scr, qt_scr, k_scr, vt_scr, wot_scr, ot_scr,
               s_scr, m_scr, g_scr, o_scr, xsem, wsem):
        i = pl.program_id(0)
        ws, wos = (awqkv_hbm, bwqkv_hbm), (awo_hbm, bwo_hbm)

        def x_copy(c):
            cols = pl.ds(pl.multiple_of(c * CH, CH), CH)
            return pltpu.make_async_copy(x_hbm.at[:, cols], x_scr.at[:, cols], xsem.at[c])

        def w_copy(src, mi):
            return pltpu.make_async_copy(src, w_scr.at[mi], wsem.at[mi])

        def wo_copy(src, mi):
            return pltpu.make_async_copy(src, wo_scr.at[mi], wsem.at[2 + mi])

        def load_qm(qi, h):
            row = lax.broadcasted_iota(jnp.int32, (128, TQ), 0)
            s0 = pl.multiple_of((h // 4) * 128, 128)
            qs = qt_scr[pl.ds(s0, 128), pl.ds(pl.multiple_of(qi * TQ, TQ), TQ)]
            return jnp.where(row // HP == (h % 4), qs, jnp.zeros_like(qs))

        def qk_chunk(c, slab, qm, u, mp):
            s = jnp.dot(k_scr[slab, c * CK:(c + 1) * CK, :], qm[:, u * SQ:(u + 1) * SQ],
                        preferred_element_type=F32)
            s_scr[c * CK:(c + 1) * CK, u * SQ:(u + 1) * SQ] = s
            mc = jnp.max(s.reshape(CK // 8, 8, SQ), axis=0)
            return mc if mp is None else jnp.maximum(mp, mc)

        def store_m(mps):
            for u, mp in enumerate(mps):
                m_scr[:, u * SQ:(u + 1) * SQ] = mp

        def prep(mi, carry):
            w_copy(awqkv_hbm, mi).wait()
            for j in range(0, F3, 128):
                n = min(128, F3 - j)
                wt_scr[j:j + n, :] = w_scr[mi, :, j:j + n].astype(F32).T.astype(BF16)
            row = lax.broadcasted_iota(jnp.int32, (DP, CH), 0) % HP
            irows = pl.ds(pl.multiple_of(mi * DP, DP), DP)

            def chunk(c, carry):
                @pl.when(mi == 0)
                def _():
                    x_copy(c).wait()
                cols = pl.ds(pl.multiple_of(c * CH, CH), CH)
                y_scr[...] = jnp.dot(wt_scr[...], x_scr[:, cols], preferred_element_type=F32)
                full = slice(None)
                qt_scr[irows, cols] = (_pad_heads(y_scr, 0, full) * QSCALE).astype(BF16)
                kp = jnp.where(row < DH, _pad_heads(y_scr, D, full), 0.0)
                for j in range(NSLAB):
                    k_scr[mi * NSLAB + j, cols, :] = kp[j * 128:(j + 1) * 128].T.astype(BF16)
                vp = _pad_heads(y_scr, 2 * D, full)
                vp = jnp.where(row < DH, vp, jnp.where(row == DH, 1.0, 0.0))
                vt_scr[irows, cols] = vp.astype(BF16)
                g_scr[:, cols] = jax.nn.sigmoid(y_scr[F3:F3 + 8, :])
                return carry

            lax.fori_loop(0, NCH, chunk, 0)
            wo_copy(awo_hbm, mi).wait()
            y_scr[0:D, 0:D] = wo_scr[mi].astype(F32)
            rw = lax.broadcasted_iota(jnp.int32, (DP, D), 0) % HP
            wop = jnp.where(rw < DH, _pad_heads(y_scr, 0, slice(0, D)), 0.0)
            for j in range(NSLAB):
                wot_scr[:, pl.ds(pl.multiple_of(mi * DP + j * 128, 128), 128)] = (
                    wop[j * 128:(j + 1) * 128].T.astype(BF16))
            return carry

        @pl.when(i == 0)
        def _():
            w_copy(ws[0], 0).start()
            for c in range(NCH):
                x_copy(c).start()
            w_copy(ws[1], 1).start()
            for mi in range(2):
                wo_copy(wos[mi], mi).start()
            wt_scr[F3:FR, :] = jnp.broadcast_to(gw_ref[...], (GR, D))
            o_scr[...] = jnp.ones((HP, TQ), F32)
            lax.fori_loop(0, 2, prep, 0)
            qm = load_qm(0, 0)
            mps = [None] * NU
            for c in range(NC):
                for u in range(NU):
                    mps[u] = qk_chunk(c, 0, qm, u, mps[u])
            store_m(mps)

        q0 = pl.multiple_of(i * TQ, TQ)

        def normalize(h, os_):
            r0 = pl.multiple_of(h * HP, HP)
            for u in range(NU):
                o = os_[u]
                l = o[DH:DH + 1, :]
                g = g_scr[0:1, pl.ds(q0 + u * SQ, SQ)]
                gg = jnp.where(h < H, g, 1.0 - g)
                ot_scr[pl.ds(r0, HP), u * SQ:(u + 1) * SQ] = (o * (gg / l)).astype(BF16)

        def half(h, with_qk):
            if with_qk:
                hn = jnp.where(h == NT_ - 1, 0, h + 1)
                qn = jnp.where(h == NT_ - 1, jnp.minimum(i + 1, NQ - 1), i)
                qm = load_qm(qn, hn)
                slabn = hn // 4
            r0 = pl.multiple_of(h * HP, HP)
            m = jnp.max(m_scr[...], axis=0, keepdims=True)
            if defer:
                normalize((h + NT_ - 1) % NT_, [o_scr[:, u * SQ:(u + 1) * SQ] for u in range(NU)])
            mps, os_ = [None] * NU, [None] * NU
            for c in range(NC):
                for u in range(NU):
                    s = s_scr[c * CK:(c + 1) * CK, u * SQ:(u + 1) * SQ]
                    p = jnp.exp2(s - m[:, u * SQ:(u + 1) * SQ]).astype(BF16)
                    oc = jnp.dot(vt_scr[pl.ds(r0, HP), c * CK:(c + 1) * CK], p, preferred_element_type=F32)
                    os_[u] = oc if os_[u] is None else os_[u] + oc
                    if with_qk:
                        mps[u] = qk_chunk(c, slabn, qm, u, mps[u])
            if with_qk:
                store_m(mps)
            if defer:
                for u in range(NU):
                    o_scr[:, u * SQ:(u + 1) * SQ] = os_[u]
            else:
                normalize(h, os_)

        def body(h, carry):
            half(h, True)
            return carry

        lax.fori_loop(0, jnp.where(i == NQ - 1, NT_ - 1, NT_), body, 0)

        @pl.when(i == NQ - 1)
        def _():
            half(NT_ - 1, False)

        if defer:
            normalize(NT_ - 1, [o_scr[:, u * SQ:(u + 1) * SQ] for u in range(NU)])
        out_ref[...] = jnp.dot(wot_scr[...], ot_scr[...], preferred_element_type=F32).astype(out_ref.dtype)

    def run(A_x, A_wqkv, A_wo, B_x, B_wqkv, B_wo, gate_w):
        del B_x
        hbm = pl.BlockSpec(memory_space=pl.ANY)
        out = pl.pallas_call(
            kernel,
            grid=(NQ,),
            in_specs=[hbm] * 5 + [pl.BlockSpec((1, D), lambda i: (0, 0))],
            out_specs=pl.BlockSpec((D, TQ), lambda i: (0, i)),
            out_shape=jax.ShapeDtypeStruct((D, S), BF16),
            scratch_shapes=[
                pltpu.VMEM((D, S), BF16),
                pltpu.VMEM((2, D, F3), BF16),
                pltpu.VMEM((2, D, D), BF16),
                pltpu.VMEM((FR, D), BF16),
                pltpu.VMEM((FR, CH), F32),
                pltpu.VMEM((2 * DP, S), BF16),
                pltpu.VMEM((2 * NSLAB, S, 128), BF16),
                pltpu.VMEM((2 * DP, S), BF16),
                pltpu.VMEM((D, 2 * DP), BF16),
                pltpu.VMEM((2 * DP, TQ), BF16),
                pltpu.VMEM((S, TQ), F32),
                pltpu.VMEM((8, TQ), F32),
                pltpu.VMEM((8, S), F32),
                pltpu.VMEM((HP, TQ), F32),
                pltpu.SemaphoreType.DMA((NCH,)),
                pltpu.SemaphoreType.DMA((4,)),
            ],
            compiler_params=pltpu.CompilerParams(
                dimension_semantics=("arbitrary",),
                vmem_limit_bytes=100 * 1024 * 1024, flags=flags),
        )(A_x.reshape(S, D).T, A_wqkv, A_wo, B_wqkv, B_wo, gate_w.reshape(1, D))
        return out.T.reshape(1, S, D)

    return run


_run = make_kernel()


@jax.jit
def pallas_gated_mix__mha_block__softmax_full_mha__prompt_kernel(
    A_x: jax.Array,
    A_wqkv: jax.Array,
    A_wo: jax.Array,
    B_x: jax.Array,
    B_wqkv: jax.Array,
    B_wo: jax.Array,
    gate_w: jax.Array,
):
    return _run(A_x, A_wqkv, A_wo, B_x, B_wqkv, B_wo, gate_w)
```

```python
import jax
import jax.numpy as jnp
from jax import lax
import jax.experimental.pallas as pl
import jax.experimental.pallas.tpu as pltpu

S, D, H, DH = 2048, 448, 16, 28
HP = 32
DP = H * HP
NSLAB = DP // 128
F3 = 3 * D
GR = 16
FR = F3 + GR
QSCALE = float(DH ** -0.5 * 1.4426950408889634)
F32, BF16 = jnp.float32, jnp.bfloat16


def _pad_heads(ref, base, cols):
    return jnp.concatenate([ref[pl.ds(base + DH * h, HP), cols] for h in range(H)], axis=0)


def make_kernel(TQ=1024, SQ=512, CK=128, CH=512, flags=None, defer=True, NP=4, WP=(0, 512, F3)):
    NW = len(WP) - 1
    PW = TQ // NP
    NQ = S // TQ
    NC = S // CK
    NT_ = 2 * H
    NCH = S // CH
    NU = TQ // SQ

    def kernel(x_hbm, awqkv_hbm, awo_hbm, bwqkv_hbm, bwo_hbm, gw_ref, out_hbm,
               x_scr, w_scr, wo_scr, wt_scr, y_scr, qt_scr, k_scr, vt_scr, wot_scr, ot_scr,
               s_scr, m_scr, g_scr, o_scr, out_scr, xsem, wsem, osem):
        i = pl.program_id(0)
        ws, wos = (awqkv_hbm, bwqkv_hbm), (awo_hbm, bwo_hbm)

        def x_copy(c):
            cols = pl.ds(pl.multiple_of(c * CH, CH), CH)
            return pltpu.make_async_copy(x_hbm.at[:, cols], x_scr.at[:, cols], xsem.at[c])

        def w_copy(src, mi, k):
            lo, hi = WP[k], WP[k + 1]
            return pltpu.make_async_copy(src.at[:, lo:hi], w_scr.at[mi, :, lo:hi], wsem.at[mi * NW + k])

        def wo_copy(src, mi):
            return pltpu.make_async_copy(src, wo_scr.at[mi * D:(mi + 1) * D, :], wsem.at[2 * NW + mi])

        def load_qm(qi, h):
            return qt_scr[pl.ds(pl.multiple_of(h * HP, HP), HP), pl.ds(pl.multiple_of(qi * TQ, TQ), TQ)]

        def qk_chunk(c, slab, qm, u, mp):
            s = jnp.dot(k_scr[slab, c * CK:(c + 1) * CK, :], qm[:, u * SQ:(u + 1) * SQ],
                        preferred_element_type=F32)
            s_scr[c * CK:(c + 1) * CK, u * SQ:(u + 1) * SQ] = s
            mc = jnp.max(s.reshape(CK // 8, 8, SQ), axis=0)
            return mc if mp is None else jnp.maximum(mp, mc)

        def store_m(mps):
            for u, mp in enumerate(mps):
                m_scr[:, u * SQ:(u + 1) * SQ] = mp

        row = lax.broadcasted_iota(jnp.int32, (DP, CH), 0) % HP

        def post(mi, cols):
            irows = pl.ds(pl.multiple_of(mi * DP, DP), DP)
            full = slice(None)
            qt_scr[irows, cols] = (_pad_heads(y_scr, 0, full) * QSCALE).astype(BF16)
            kp = jnp.where(row < DH, _pad_heads(y_scr, D, full), 0.0)
            for h in range(H):
                k_scr[mi * H + h, cols, :] = kp[h * HP:(h + 1) * HP].T.astype(BF16)
            vp = _pad_heads(y_scr, 2 * D, full)
            vp = jnp.where(row < DH, vp, jnp.where(row == DH, 1.0, 0.0))
            vt_scr[irows, cols] = vp.astype(BF16)
            g_scr[:, cols] = jax.nn.sigmoid(y_scr[F3:F3 + 8, :])

        def project(mi, carry):
            def chunk(c, carry):
                @pl.when(mi == 0)
                def _():
                    x_copy(c).wait()
                cols = pl.ds(pl.multiple_of(c * CH, CH), CH)
                y_scr[...] = jnp.dot(wt_scr[...], x_scr[:, cols], preferred_element_type=F32)
                post(mi, cols)
                return carry

            lax.fori_loop(1 - mi, NCH, chunk, 0)

            @pl.when(mi == 0)
            def _():
                for k in range(NW):
                    w_copy(ws[1], 1, k).wait()
                for kk in range(2):
                    wo_copy(wos[kk], kk).wait()
                for j in range(0, F3, 128):
                    n = min(128, F3 - j)
                    wt_scr[j:j + n, :] = w_scr[1, :, j:j + n].T
                for j in range(2 * D // 128):
                    wot_scr[:, j * 128:(j + 1) * 128] = wo_scr[j * 128:(j + 1) * 128, :].T
                qm = load_qm(0, 0)
                mps = [None] * NU
                for c in range(NC):
                    for u in range(NU):
                        mps[u] = qk_chunk(c, 0, qm, u, mps[u])
                store_m(mps)
            return carry

        @pl.when(i == 0)
        def _():
            x_copy(0).start()
            for k in range(NW):
                w_copy(ws[0], 0, k).start()
            wt_scr[F3:FR, :] = jnp.broadcast_to(gw_ref[...].reshape(1, D), (GR, D))
            o_scr[...] = jnp.ones((HP, TQ), F32)
            for k in range(NW):
                if k == 1:
                    for c in range(1, NCH):
                        x_copy(c).start()
                    for kk in range(NW):
                        w_copy(ws[1], 1, kk).start()
                    for kk in range(2):
                        wo_copy(wos[kk], kk).start()
                w_copy(ws[0], 0, k).wait()
                for j in range(WP[k], WP[k + 1], 128):
                    n = min(128, F3 - j)
                    wt_scr[j:j + n, :] = w_scr[0, :, j:j + n].T
                if k == 0:
                    x_copy(0).wait()
                hi = FR if k == NW - 1 else WP[k + 1]
                y_scr[WP[k]:hi, :] = jnp.dot(wt_scr[WP[k]:hi, :], x_scr[:, 0:CH], preferred_element_type=F32)
            post(0, slice(0, CH))
            lax.fori_loop(0, 2, project, 0)

        q0 = pl.multiple_of(i * TQ, TQ)

        def normalize(h, os_):
            for u in range(NU):
                o = os_[u]
                l = o[DH:DH + 1, :]
                g = g_scr[0:1, pl.ds(q0 + u * SQ, SQ)]
                gg = jnp.where(h < H, g, 1.0 - g)
                ot_scr[pl.ds(pl.multiple_of(h * HP, HP), HP), u * SQ:(u + 1) * SQ] = o * (gg / l)

        def half(h, with_qk):
            if with_qk:
                tn = i * NT_ + h + 1
                slabn = tn & (NT_ - 1)
                qm = load_qm(tn >> 5, slabn)
            r0 = pl.multiple_of(h * HP, HP)
            m = jnp.max(m_scr[...], axis=0, keepdims=True)
            if defer:
                normalize((h + NT_ - 1) & (NT_ - 1), [o_scr[:, u * SQ:(u + 1) * SQ] for u in range(NU)])
            mps, os_ = [None] * NU, [None] * NU
            for c in range(NC):
                for u in range(NU):
                    s = s_scr[c * CK:(c + 1) * CK, u * SQ:(u + 1) * SQ]
                    p = jnp.exp2(s - m[:, u * SQ:(u + 1) * SQ]).astype(BF16)
                    oc = jnp.dot(vt_scr[pl.ds(r0, HP), c * CK:(c + 1) * CK], p, preferred_element_type=F32)
                    os_[u] = oc if os_[u] is None else os_[u] + oc
                    if with_qk:
                        mps[u] = qk_chunk(c, slabn, qm, u, mps[u])
            if with_qk:
                store_m(mps)
            if defer:
                for u in range(NU):
                    o_scr[:, u * SQ:(u + 1) * SQ] = os_[u]
            else:
                normalize(h, os_)

        def body(h, carry):
            half(h, True)
            return carry

        lax.fori_loop(0, jnp.where(i == NQ - 1, NT_ - 1, NT_), body, 0)

        def out_copy(qi, p):
            return pltpu.make_async_copy(
                out_scr.at[qi, :, p * PW:(p + 1) * PW],
                out_hbm.at[:, pl.ds(pl.multiple_of(qi * TQ + p * PW, PW), PW)], osem.at[qi * NP + p])

        def out_proj():
            normalize(NT_ - 1, [o_scr[:, u * SQ:(u + 1) * SQ] for u in range(NU)])
            prow = lax.broadcasted_iota(jnp.int32, (2 * DH, PW), 0)
            for p in range(NP):
                cs = slice(p * PW, (p + 1) * PW)
                oc = jnp.concatenate(
                    [jnp.where(prow < DH, ot_scr[2 * HP * t:2 * HP * t + 2 * DH, cs],
                               ot_scr[2 * HP * t + HP - DH:2 * HP * t + HP + DH, cs]) for t in range(H)], axis=0)
                y = jnp.dot(wot_scr[...], oc.astype(BF16), preferred_element_type=F32)
                out_scr[i, :, p * PW:(p + 1) * PW] = y.astype(BF16)
                out_copy(i, p).start()

        @pl.when(i < NQ - 1)
        def _():
            out_proj()

        @pl.when(i == NQ - 1)
        def _():
            half(NT_ - 1, False)
            out_proj()
            for qi in range(NQ):
                for p in range(NP):
                    out_copy(qi, p).wait()

    def run(A_x, A_wqkv, A_wo, B_x, B_wqkv, B_wo, gate_w):
        del B_x
        hbm = pl.BlockSpec(memory_space=pl.ANY)
        out = pl.pallas_call(
            kernel,
            grid=(NQ,),
            in_specs=[hbm] * 5 + [pl.BlockSpec((D,), lambda i: (0,))],
            out_specs=hbm,
            out_shape=jax.ShapeDtypeStruct((D, S), BF16),
            scratch_shapes=[
                pltpu.VMEM((D, S), BF16),
                pltpu.VMEM((2, D, F3), BF16),
                pltpu.VMEM((2 * D, D), BF16),
                pltpu.VMEM((FR, D), BF16),
                pltpu.VMEM((FR, CH), F32),
                pltpu.VMEM((2 * DP, S), BF16),
                pltpu.VMEM((2 * H, S, HP), BF16),
                pltpu.VMEM((2 * DP, S), BF16),
                pltpu.VMEM((D, 2 * D), BF16),
                pltpu.VMEM((2 * DP + 8, TQ), F32),
                pltpu.VMEM((S, TQ), F32),
                pltpu.VMEM((8, TQ), F32),
                pltpu.VMEM((8, S), F32),
                pltpu.VMEM((HP, TQ), F32),
                pltpu.VMEM((NQ, D, TQ), BF16),
                pltpu.SemaphoreType.DMA((NCH,)),
                pltpu.SemaphoreType.DMA((2 * NW + 2,)),
                pltpu.SemaphoreType.DMA((NQ * NP,)),
            ],
            compiler_params=pltpu.CompilerParams(
                dimension_semantics=("arbitrary",),
                vmem_limit_bytes=100 * 1024 * 1024, flags=flags),
        )(A_x.reshape(S, D).T, A_wqkv, A_wo, B_wqkv, B_wo, gate_w)
        return out.T.reshape(1, S, D)

    return run


_run = make_kernel()


@jax.jit
def pallas_gated_mix__mha_block__softmax_full_mha__prompt_kernel(
    A_x: jax.Array,
    A_wqkv: jax.Array,
    A_wo: jax.Array,
    B_x: jax.Array,
    B_wqkv: jax.Array,
    B_wo: jax.Array,
    gate_w: jax.Array,
):
    return _run(A_x, A_wqkv, A_wo, B_x, B_wqkv, B_wo, gate_w)
```

```python
import jax
import jax.numpy as jnp
from jax import lax
import jax.experimental.pallas as pl
import jax.experimental.pallas.tpu as pltpu

S, D, H, DH = 2048, 448, 16, 28
HP = 32
DP = H * HP
F3 = 3 * D
GR = 16
FR = F3 + GR
QSCALE = float(DH ** -0.5 * 1.4426950408889634)
F32, BF16 = jnp.float32, jnp.bfloat16


def _pad_heads(ref, base, cols):
    return jnp.concatenate([ref[pl.ds(base + DH * h, HP), cols] for h in range(H)], axis=0)


def make_kernel(TQ=1024, SQ=512, CK=128, CH=512, NP=4, PRE_AT=(1, 5, 9, 13), WP=(0, 512, F3)):
    NW = len(WP) - 1
    PW = TQ // NP
    NQ = S // TQ
    NC = S // CK
    NT_ = 2 * H
    NCH = S // CH
    NU = TQ // SQ

    def kernel(x_hbm, awqkv_hbm, awo_hbm, bwqkv_hbm, bwo_hbm, gw_ref, out_hbm,
               x_scr, w_scr, wo_scr, wt_scr, y_scr, qt_scr, k_scr, vt_scr, wot_scr, ot_scr,
               s_scr, m_scr, g_scr, o_scr, part_scr, out_scr, xsem, wsem, osem):
        i = pl.program_id(0)
        ws, wos = (awqkv_hbm, bwqkv_hbm), (awo_hbm, bwo_hbm)

        def x_copy(c):
            cols = pl.ds(pl.multiple_of(c * CH, CH), CH)
            return pltpu.make_async_copy(x_hbm.at[:, cols], x_scr.at[:, cols], xsem.at[c])

        def w_copy(src, mi, k):
            lo, hi = WP[k], WP[k + 1]
            return pltpu.make_async_copy(src.at[:, lo:hi], w_scr.at[mi, :, lo:hi], wsem.at[mi * NW + k])

        def wo_copy(src, mi):
            return pltpu.make_async_copy(src, wo_scr.at[mi * D:(mi + 1) * D, :], wsem.at[2 * NW + mi])

        def load_qm(qi, h):
            return qt_scr[pl.ds(pl.multiple_of(h * HP, HP), HP), pl.ds(pl.multiple_of(qi * TQ, TQ), TQ)]

        def qk_chunk(c, hd, qm, u, mp):
            s = jnp.dot(k_scr[hd, c * CK:(c + 1) * CK, :], qm[:, u * SQ:(u + 1) * SQ],
                        preferred_element_type=F32)
            s_scr[c * CK:(c + 1) * CK, u * SQ:(u + 1) * SQ] = s
            mc = jnp.max(s.reshape(CK // 8, 8, SQ), axis=0)
            return mc if mp is None else jnp.maximum(mp, mc)

        def store_m(mps):
            for u, mp in enumerate(mps):
                m_scr[:, u * SQ:(u + 1) * SQ] = mp

        row = lax.broadcasted_iota(jnp.int32, (DP, CH), 0) % HP

        def post(mi, cols):
            irows = pl.ds(pl.multiple_of(mi * DP, DP), DP)
            full = slice(None)
            qt_scr[irows, cols] = (_pad_heads(y_scr, 0, full) * QSCALE).astype(BF16)
            kp = jnp.where(row < DH, _pad_heads(y_scr, D, full), 0.0)
            for h in range(H):
                k_scr[mi * H + h, cols, :] = kp[h * HP:(h + 1) * HP].T.astype(BF16)
            vp = _pad_heads(y_scr, 2 * D, full)
            vp = jnp.where(row < DH, vp, jnp.where(row == DH, 1.0, 0.0))
            vt_scr[irows, cols] = vp.astype(BF16)
            g_scr[:, cols] = jax.nn.sigmoid(y_scr[F3:F3 + 8, :])

        def project(mi, carry):
            def chunk(c, carry):
                @pl.when(mi == 0)
                def _():
                    x_copy(c).wait()
                cols = pl.ds(pl.multiple_of(c * CH, CH), CH)
                y_scr[...] = jnp.dot(wt_scr[...], x_scr[:, cols], preferred_element_type=F32)
                post(mi, cols)
                return carry

            lax.fori_loop(1 - mi, NCH, chunk, 0)

            @pl.when(mi == 0)
            def _():
                for k in range(NW):
                    w_copy(ws[1], 1, k).wait()
                for kk in range(2):
                    wo_copy(wos[kk], kk).wait()
                for j in range(0, F3, 128):
                    n = min(128, F3 - j)
                    wt_scr[j:j + n, :] = w_scr[1, :, j:j + n].T
                for j in range(2 * D // 128):
                    wot_scr[:, j * 128:(j + 1) * 128] = wo_scr[j * 128:(j + 1) * 128, :].T
                qm = load_qm(0, 0)
                mps = [None] * NU
                for c in range(NC):
                    for u in range(NU):
                        mps[u] = qk_chunk(c, 0, qm, u, mps[u])
                store_m(mps)
            return carry

        @pl.when(i == 0)
        def _():
            x_copy(0).start()
            for k in range(NW):
                w_copy(ws[0], 0, k).start()
            wt_scr[F3:FR, :] = jnp.broadcast_to(gw_ref[...].reshape(1, D), (GR, D))
            o_scr[...] = jnp.ones((HP, TQ), F32)
            for k in range(NW):
                if k == 1:
                    for c in range(1, NCH):
                        x_copy(c).start()
                    for kk in range(NW):
                        w_copy(ws[1], 1, kk).start()
                    for kk in range(2):
                        wo_copy(wos[kk], kk).start()
                w_copy(ws[0], 0, k).wait()
                for j in range(WP[k], WP[k + 1], 128):
                    n = min(128, F3 - j)
                    wt_scr[j:j + n, :] = w_scr[0, :, j:j + n].T
                if k == 0:
                    x_copy(0).wait()
                hi = FR if k == NW - 1 else WP[k + 1]
                y_scr[WP[k]:hi, :] = jnp.dot(wt_scr[WP[k]:hi, :], x_scr[:, 0:CH], preferred_element_type=F32)
            post(0, slice(0, CH))
            lax.fori_loop(0, 2, project, 0)

        q0 = pl.multiple_of(i * TQ, TQ)

        def normalize(h):
            for u in range(NU):
                o = o_scr[:, u * SQ:(u + 1) * SQ]
                l = o[DH:DH + 1, :]
                g = g_scr[0:1, pl.ds(q0 + u * SQ, SQ)]
                gg = jnp.where(h < H, g, 1.0 - g)
                ot_scr[pl.ds(pl.multiple_of(h * HP, HP), HP), u * SQ:(u + 1) * SQ] = o * (gg / l)

        def half(h, with_qk, extra=None):
            if with_qk:
                tn = i * NT_ + h + 1
                hn = tn & (NT_ - 1)
                qm = load_qm(tn >> 5, hn)
            r0 = pl.multiple_of(h * HP, HP)
            m = jnp.max(m_scr[...], axis=0, keepdims=True)
            normalize((h + NT_ - 1) & (NT_ - 1))
            mps, os_ = [None] * NU, [None] * NU
            for c in range(NC):
                for u in range(NU):
                    s = s_scr[c * CK:(c + 1) * CK, u * SQ:(u + 1) * SQ]
                    p = jnp.exp2(s - m[:, u * SQ:(u + 1) * SQ]).astype(BF16)
                    oc = jnp.dot(vt_scr[pl.ds(r0, HP), c * CK:(c + 1) * CK], p, preferred_element_type=F32)
                    os_[u] = oc if os_[u] is None else os_[u] + oc
                    if with_qk:
                        mps[u] = qk_chunk(c, hn, qm, u, mps[u])
                if extra is not None:
                    extra(c)
            if with_qk:
                store_m(mps)
            for u in range(NU):
                o_scr[:, u * SQ:(u + 1) * SQ] = os_[u]

        def body(h, carry):
            half(h, True)
            return carry

        lax.fori_loop(0, jnp.where(i == NQ - 1, NT_ - 1, NT_), body, 0)

        def out_copy(qi, p):
            return pltpu.make_async_copy(
                out_scr.at[qi, :, p * PW:(p + 1) * PW],
                out_hbm.at[:, pl.ds(pl.multiple_of(qi * TQ + p * PW, PW), PW)], osem.at[qi * NP + p])

        def compact(t0, t1, cs):
            prow = lax.broadcasted_iota(jnp.int32, (2 * DH, cs.stop - cs.start), 0)
            return jnp.concatenate(
                [jnp.where(prow < DH, ot_scr[2 * HP * t:2 * HP * t + 2 * DH, cs],
                           ot_scr[2 * HP * t + HP - DH:2 * HP * t + HP + DH, cs]) for t in range(t0, t1)],
                axis=0).astype(BF16)

        KS = 768

        def partial_proj(c):
            if c in PRE_AT:
                p = PRE_AT.index(c)
                cs = slice(p * 128, (p + 1) * 128)
                part_scr[:, cs] = jnp.dot(wot_scr[:, 0:KS], compact(0, 14, cs)[0:KS], preferred_element_type=F32)

        def out_proj(partial=False):
            normalize(NT_ - 1)
            for p in range(NP):
                cs = slice(p * PW, (p + 1) * PW)
                if partial and (p + 1) * PW <= 128 * len(PRE_AT):
                    oc = compact(12, 16, cs)[KS - 12 * 2 * DH:]
                    y = part_scr[:, cs] + jnp.dot(wot_scr[:, KS:], oc, preferred_element_type=F32)
                else:
                    y = jnp.dot(wot_scr[...], compact(0, H, cs), preferred_element_type=F32)
                out_scr[i, :, cs] = y.astype(BF16)
                out_copy(i, p).start()

        @pl.when(i < NQ - 1)
        def _():
            out_proj()

        @pl.when(i == NQ - 1)
        def _():
            half(NT_ - 1, False, partial_proj)
            out_proj(True)
            for qi in range(NQ):
                for p in range(NP):
                    out_copy(qi, p).wait()

    def run(A_x, A_wqkv, A_wo, B_x, B_wqkv, B_wo, gate_w):
        del B_x
        hbm = pl.BlockSpec(memory_space=pl.ANY)
        out = pl.pallas_call(
            kernel,
            grid=(NQ,),
            in_specs=[hbm] * 5 + [pl.BlockSpec((D,), lambda i: (0,))],
            out_specs=hbm,
            out_shape=jax.ShapeDtypeStruct((D, S), BF16),
            scratch_shapes=[
                pltpu.VMEM((D, S), BF16),
                pltpu.VMEM((2, D, F3), BF16),
                pltpu.VMEM((2 * D, D), BF16),
                pltpu.VMEM((FR, D), BF16),
                pltpu.VMEM((FR, CH), F32),
                pltpu.VMEM((2 * DP, S), BF16),
                pltpu.VMEM((2 * H, S, HP), BF16),
                pltpu.VMEM((2 * DP, S), BF16),
                pltpu.VMEM((D, 2 * D), BF16),
                pltpu.VMEM((2 * DP + 8, TQ), F32),
                pltpu.VMEM((S, TQ), F32),
                pltpu.VMEM((8, TQ), F32),
                pltpu.VMEM((8, S), F32),
                pltpu.VMEM((HP, TQ), F32),
                pltpu.VMEM((D, 128 * len(PRE_AT)), F32),
                pltpu.VMEM((NQ, D, TQ), BF16),
                pltpu.SemaphoreType.DMA((NCH,)),
                pltpu.SemaphoreType.DMA((2 * NW + 2,)),
                pltpu.SemaphoreType.DMA((NQ * NP,)),
            ],
            compiler_params=pltpu.CompilerParams(
                dimension_semantics=("arbitrary",),
                vmem_limit_bytes=100 * 1024 * 1024),
        )(A_x.reshape(S, D).T, A_wqkv, A_wo, B_wqkv, B_wo, gate_w)
        return out.T.reshape(1, S, D)

    return run


_run = make_kernel()


@jax.jit
def pallas_gated_mix__mha_block__softmax_full_mha__prompt_kernel(
    A_x: jax.Array,
    A_wqkv: jax.Array,
    A_wo: jax.Array,
    B_x: jax.Array,
    B_wqkv: jax.Array,
    B_wo: jax.Array,
    gate_w: jax.Array,
):
    return _run(A_x, A_wqkv, A_wo, B_x, B_wqkv, B_wo, gate_w)
```
